```python
import os as _os
_os.environ.setdefault("JAX_PLATFORMS", "cpu")
import jax
import jax.numpy as jnp

def _softmax(x, axis=-1):
    return jax.nn.softmax(x, axis=axis)
def _gelu(x):
    return jax.nn.gelu(x, approximate=True)
def _silu(x):
    return jax.nn.silu(x)
def _sigmoid(x):
    return jax.nn.sigmoid(x)
def _layernorm(x, axis=-1, eps=1e-5):
    m = jnp.mean(x, axis=axis, keepdims=True)
    v = jnp.var(x, axis=axis, keepdims=True)
    return (x - m) / jnp.sqrt(v + eps)
def _scatter_add(tgt, idx, src, axis=0):
    return tgt.at[idx].add(src)
def _segment_sum(src, seg, n):
    return jax.ops.segment_sum(src, seg, n)
class _Rng:
    def __init__(self, key):
        self._k = key
    def _next(self):
        self._k, sub = jax.random.split(self._k)
        return sub
    def normal(self, shape):
        return jax.random.normal(self._next(), shape, dtype=jnp.bfloat16)
    def randint(self, lo, hi, shape):
        return jax.random.randint(self._next(), shape, lo, hi, dtype=jnp.int32)
    def uniform(self, shape, lo=0.0, hi=1.0):
        return jax.random.uniform(self._next(), shape, jnp.bfloat16, lo, hi)
    def permutation(self, n):
        return jax.random.permutation(self._next(), n)


kernel_name = 'standalone__gqa_block_cached__near_ridge'

def setup_inputs():
    _rng = _Rng(jax.random.key(int.from_bytes(__import__("os").urandom(4), "little")))
    _w = (lambda a: (lambda t: t.astype(jnp.bfloat16) if jnp.issubdtype(t.dtype, jnp.floating) else t)(jnp.asarray(a)))
    B, Sq, D = 8, 96, 448
    Hq, Hkv, Sk, Dh = 16, 8, 2048, 256
    assert Hq % Hkv == 0, (Hq, Hkv)
    return {
        "x": _w((lambda *s: _rng.normal(s) * 0.8)(B, Sq, D)),
        "k_cache": _w((lambda *s: _rng.normal(s) * 0.8)(B, Hkv, Sk, Dh)),
        "v_cache": _w((lambda *s: _rng.normal(s) * 0.05)(B, Hkv, Sk, Dh)),
        "wq": _w((lambda *s: _rng.normal(s) * 0.8)(D, Hq * Dh) * (D ** -0.5)),
        "wo": _w((lambda *s: _rng.normal(s) * 0.05)(Hq * Dh, D) * ((Hq * Dh) ** -0.5)),
    }

def reference(x, k_cache, v_cache, wq, wo):
    B, Sq, D = x.shape
    Hq, Dh = 16, 256
    Hkv = k_cache.shape[1]
    rep = Hq // Hkv
    q = (lambda x, *d: x.transpose(*d))((x @ wq).reshape(B, Sq, Hq, Dh), 0, 2, 1, 3)
    k = jnp.repeat(k_cache, rep, axis=1)
    v = jnp.repeat(v_cache, rep, axis=1)
    scores = jnp.einsum("bhqd,bhkd->bhqk", q, k) * (Dh ** -0.5)
    p = _softmax(scores, axis=-1)
    o = jnp.einsum("bhqk,bhkd->bhqd", p, v)
    return (lambda x, *d: x.transpose(*d))(o, 0, 2, 1, 3).reshape(B, Sq, Hq * Dh) @ wo
```

```python
import functools
import jax, jax.numpy as jnp
from jax import lax
import jax.experimental.pallas as pl
import jax.experimental.pallas.tpu as pltpu

B, SQ, D, HQ, HKV, SK, DH = 8, 96, 448, 16, 8, 2048, 256
REP = HQ // HKV
M = REP * SQ
NU = B * HKV
LOG2E = 1.4426950408889634

def make(nbuf=4, order="QSOP", nodma=False, exp2=True, unroll=1):
    GW = REP * DH

    def kern(x_hbm, k_hbm, v_hbm, wq_hbm, wo_hbm, o_hbm,
             xbuf, wqbuf, wobuf, kbuf, vbuf, qbuf, sbuf, mbuf, obuf, acc, outbuf,
             xsem, wqsem, wosem, ksem, vsem, osem):
        def k_copy(u):
            return pltpu.make_async_copy(k_hbm.at[u % B, u // B], kbuf.at[u % nbuf], ksem.at[u % nbuf])
        def v_copy(u):
            return pltpu.make_async_copy(v_hbm.at[u % B, u // B], vbuf.at[u % nbuf], vsem.at[u % nbuf])
        def wq_copy(h):
            return pltpu.make_async_copy(wq_hbm.at[:, pl.ds(h * GW, GW)], wqbuf.at[h], wqsem.at[h])
        def wo_copy(h):
            return pltpu.make_async_copy(wo_hbm.at[:, pl.ds(h * GW, GW)], wobuf.at[h], wosem.at[h])
        def x_copy():
            return pltpu.make_async_copy(x_hbm, xbuf, xsem.at[0])
        def o_copy(b):
            return pltpu.make_async_copy(outbuf.at[b], o_hbm.at[b], osem.at[b])

        qscale = (DH ** -0.5) * (LOG2E if exp2 else 1.0)
        ex = jnp.exp2 if exp2 else jnp.exp

        def stage_q(u):
            b = u % B; h = u // B
            q = jnp.dot(xbuf[b], wqbuf[h], preferred_element_type=jnp.float32)
            q = (q * qscale).astype(jnp.bfloat16)
            qbuf[u % 2, 0:SQ, :] = q[:, :DH]
            qbuf[u % 2, SQ:M, :] = q[:, DH:]

        def stage_s(u):
            s = lax.dot_general(qbuf[u % 2], kbuf[u % nbuf], (((1,), (1,)), ((), ())), preferred_element_type=jnp.float32)
            sbuf[u % 2] = s
            m = jnp.max(s, axis=-1, keepdims=True)
            mbuf[u % 2] = jnp.broadcast_to(m, (M, 128))

        def stage_p(u):
            m = mbuf[u % 2]
            p = ex(sbuf[u % 2] - jnp.tile(m, (1, SK // 128)))
            l = jnp.sum(p, axis=-1, keepdims=True)
            o = jnp.dot(p.astype(jnp.bfloat16), vbuf[u % nbuf], preferred_element_type=jnp.float32)
            o = (o * (1.0 / l)).astype(jnp.bfloat16)
            obuf[u % 2, :, 0:DH] = o[:SQ]
            obuf[u % 2, :, DH:GW] = o[SQ:]

        def stage_o(u):
            b = u % B; h = u // B
            y = lax.dot_general(obuf[u % 2], wobuf[h], (((1,), (1,)), ((), ())), preferred_element_type=jnp.float32)
            a = acc[b] + y
            acc[b] = a
            outbuf[b] = a.astype(jnp.bfloat16)

        stages = dict(Q=(stage_q, 2), S=(stage_s, 1), P=(stage_p, 0), O=(stage_o, -1))

        x_copy().start(); wq_copy(0).start()
        for u in range(nbuf):
            k_copy(u).start(); v_copy(u).start()
            if u == 0: wo_copy(0).start()
            if u == 1:
                wq_copy(1).start(); wo_copy(1).start()
        acc[...] = jnp.zeros(acc.shape, acc.dtype)

        def iteration(i, static):
            def valid(u): return (0 <= u < NU) if static else True
            def when(c, f):
                if static:
                    if c: f()
                else:
                    pl.when(c)(f)
            if not nodma or static:
                if valid(i + 2):
                    if static and i + 2 == 0: x_copy().wait()
                    when((i + 2) % B == 0, lambda: wq_copy((i + 2) // B).wait())
                if valid(i + 1) and (not nodma or i + 1 < nbuf): k_copy(i + 1).wait()
                if valid(i) and (not nodma or i < nbuf): v_copy(i).wait()
                if valid(i - 1):
                    when((i - 1) % B == 0, lambda: wo_copy((i - 1) // B).wait())
                if valid(i - 2):
                    when((i - 2) // B == HKV - 1, lambda: o_copy((i - 2) % B).start())
                if not nodma:
                    when((i >= 0) & (i + nbuf < NU) if not static else (0 <= i and i + nbuf < NU), lambda: k_copy(i + nbuf).start())
                    when((i >= 1) & (i - 1 + nbuf < NU) if not static else (1 <= i and i - 1 + nbuf < NU), lambda: v_copy(i - 1 + nbuf).start())
                def w_start():
                    wq_copy(i // B + 2).start(); wo_copy(i // B + 2).start()
                when((i % B == 0) & (i // B + 2 < HKV) if not static else (i >= 0 and i % B == 0 and i // B + 2 < HKV), w_start)
            for c in order:
                f, d = stages[c]
                if valid(i + d): f(i + d)

        for i in range(-2, 1):
            iteration(i, True)
        lo, hi = 1, NU - 2
        if nodma:
            for h in range(2, HKV):
                if h > 2: wq_copy(h).start(); wo_copy(h).start()
            for h in range(1, HKV):
                wq_copy(h).wait(); wo_copy(h).wait()
            wo_copy(0).wait()
            for u in range(2, nbuf): k_copy(u).wait()
            for u in range(1, nbuf): v_copy(u).wait()
        lax.fori_loop(lo, hi, lambda i, c: (iteration(i, False), c)[1], 0, unroll=unroll)
        if nodma:
            for i in range(hi, NU + 1):
                for c in order:
                    f, d = stages[c]
                    if 0 <= i + d < NU: f(i + d)
            for b in range(B): o_copy(b).start()
            for b in range(B): o_copy(b).wait()
        else:
            for i in range(hi, NU + 2):
                iteration(i, True)
            for b in range(B): o_copy(b).wait()

    def fn(x, k_cache, v_cache, wq, wo):
        return pl.pallas_call(
            kern,
            in_specs=[pl.BlockSpec(memory_space=pltpu.HBM)] * 5,
            out_specs=pl.BlockSpec(memory_space=pltpu.HBM),
            out_shape=jax.ShapeDtypeStruct((B, SQ, D), jnp.bfloat16),
            scratch_shapes=[
                pltpu.VMEM((B, SQ, D), jnp.bfloat16),
                pltpu.VMEM((HKV, D, GW), jnp.bfloat16),
                pltpu.VMEM((HKV, D, GW), jnp.bfloat16),
                pltpu.VMEM((nbuf, SK, DH), jnp.bfloat16),
                pltpu.VMEM((nbuf, SK, DH), jnp.bfloat16),
                pltpu.VMEM((2, M, DH), jnp.bfloat16),
                pltpu.VMEM((2, M, SK), jnp.float32),
                pltpu.VMEM((2, M, 128), jnp.float32),
                pltpu.VMEM((2, SQ, GW), jnp.bfloat16),
                pltpu.VMEM((B, SQ, D), jnp.float32),
                pltpu.VMEM((B, SQ, D), jnp.bfloat16),
                pltpu.SemaphoreType.DMA((1,)),
                pltpu.SemaphoreType.DMA((HKV,)),
                pltpu.SemaphoreType.DMA((HKV,)),
                pltpu.SemaphoreType.DMA((nbuf,)),
                pltpu.SemaphoreType.DMA((nbuf,)),
                pltpu.SemaphoreType.DMA((B,)),
            ],
            compiler_params=pltpu.CompilerParams(vmem_limit_bytes=100 << 20),
        )(x, k_cache, v_cache, wq, wo.T)
    return fn


@jax.jit
def pallas_standalone__gqa_block_cached__near_ridge_kernel(x, k_cache, v_cache, wq, wo):
    return make(order="PSQO")(x, k_cache, v_cache, wq, wo)
```

```python
import jax
import jax.numpy as jnp
from jax import lax
import jax.experimental.pallas as pl
import jax.experimental.pallas.tpu as pltpu

B, SQ, D, HQ, HKV, SK, DH = 8, 96, 448, 16, 8, 2048, 256
REP = HQ // HKV
M = REP * SQ
NU = B * HKV
GW = REP * DH
NS = 4
AHEAD = 3
ROWS = 64
WROWS = 64


def _kernel(x_hbm, k_hbm, v_hbm, wq_hbm, wot_hbm, o_hbm,
            xbuf, wqbuf, wobuf, kbuf, vbuf, qbuf, sbuf, mbuf, obuf, acc, outbuf,
            xsem, wqsem, wosem, ksem, vsem, osem):

    def start_block(hbm, buf, sem, u, rows=ROWS):
        slot = u & (NS - 1)
        n = SK // 2 // rows
        for half in range(2):
            for j in range(n):
                r = pl.ds(half * (SK // 2) + (j // 2 + (j % 2) * (n // 2)) * rows, rows)
                pltpu.make_async_copy(hbm.at[u & 7, u >> 3, r], buf.at[slot, r],
                                      sem.at[slot]).start(priority=j % 2)

    def wait_all(buf, sem, idx):
        pltpu.make_async_copy(buf.at[idx], buf.at[idx], sem.at[idx]).wait()

    def w_copy(hbm, buf, sem, h, r0, nr):
        r = pl.ds(r0, nr)
        return pltpu.make_async_copy(hbm.at[r, pl.ds(h * GW, GW)], buf.at[h, r], sem.at[h])

    def w_whole(hbm, buf, sem, h):
        w_copy(hbm, buf, sem, h, 0, D // 2).start(priority=0)
        w_copy(hbm, buf, sem, h, D // 2, D // 2).start(priority=1)

    def x_copy(half):
        r = pl.ds(half * (B // 2), B // 2)
        return pltpu.make_async_copy(x_hbm.at[r], xbuf.at[r], xsem.at[half])

    def o_copy(b):
        return pltpu.make_async_copy(outbuf.at[b], o_hbm.at[b], osem.at[b])

    def stage_q(u):
        q = jnp.dot(xbuf[u & 7], wqbuf[u >> 3], preferred_element_type=jnp.float32)
        q = (q * (DH ** -0.5)).astype(jnp.bfloat16)
        qbuf[u & 1, 0:SQ, :] = q[:, :DH]
        qbuf[u & 1, SQ:M, :] = q[:, DH:]

    def stage_s(u):
        s = lax.dot_general(qbuf[u & 1], kbuf[u & (NS - 1)], (((1,), (1,)), ((), ())),
                            preferred_element_type=jnp.float32)
        sbuf[u & 1] = s
        mx = s[:, 0:128]
        for j in range(1, SK // 128):
            mx = jnp.maximum(mx, s[:, j * 128:(j + 1) * 128])
        mbuf[u & 1] = jnp.broadcast_to(jnp.max(mx, axis=-1, keepdims=True), (M, 128))

    def stage_p(u):
        p = jnp.exp(sbuf[u & 1] - jnp.tile(mbuf[u & 1], (1, SK // 128)))
        l = jnp.sum(p, axis=-1, keepdims=True)
        o = jnp.dot(p.astype(jnp.bfloat16), vbuf[u & (NS - 1)], preferred_element_type=jnp.float32)
        o = (o * (1.0 / l)).astype(jnp.bfloat16)
        obuf[u & 1, :, 0:DH] = o[:SQ]
        obuf[u & 1, :, DH:GW] = o[SQ:]

    def stage_o(u):
        b = u & 7
        y = lax.dot_general(obuf[u & 1], wobuf[u >> 3], (((1,), (1,)), ((), ())),
                            preferred_element_type=jnp.float32)
        a = acc[b] + y
        acc[b] = a
        outbuf[b] = a.astype(jnp.bfloat16)

    def iteration(i):
        static = isinstance(i, int)

        def valid(u):
            return (0 <= u < NU) if static else True

        def when(c, f):
            if not static:
                pl.when(c)(f)
            elif c:
                f()

        if static and i == -2:
            x_copy(0).wait()
            x_copy(1).wait()
        if static and i == -1:
            w_whole(wot_hbm, wobuf, wosem, 0)
        if valid(i + 2):
            when(((i + 2) & 7) == 0, lambda: wait_all(wqbuf, wqsem, (i + 2) >> 3))
        if valid(i - 1):
            when(((i - 1) & 7) == 0, lambda: wait_all(wobuf, wosem, (i - 1) >> 3))
        if valid(i):
            wait_all(vbuf, vsem, i & (NS - 1))
        if valid(i + 1):
            wait_all(kbuf, ksem, (i + 1) & (NS - 1))

        if valid(i - 2):
            when(((i - 2) >> 3) == HKV - 1, lambda: o_copy((i - 2) & 7).start())

        def piece(hbm, buf, sem, j, priority):
            c = ((j >> 3) + 1 < HKV) & ((j & 7) < D // WROWS)
            if static:
                c = c and j >= 0
                r0 = (j & 7) * WROWS
            else:
                r0 = pl.multiple_of((j & 7) * WROWS, WROWS)
            when(c, lambda: w_copy(hbm, buf, sem, (j >> 3) + 1, r0, WROWS).start(priority=priority))
        piece(wq_hbm, wqbuf, wqsem, i + 2, 0)
        piece(wot_hbm, wobuf, wosem, i - 1, 1)

        if valid(i + AHEAD):
            start_block(k_hbm, kbuf, ksem, i + AHEAD)
        if valid(i):
            stage_p(i)
        if valid(i + AHEAD):
            start_block(v_hbm, vbuf, vsem, i + AHEAD)
        if valid(i + 1):
            stage_s(i + 1)
        if valid(i + 2):
            stage_q(i + 2)
        if valid(i - 1):
            stage_o(i - 1)

    x_copy(0).start(priority=0)
    x_copy(1).start(priority=1)
    w_whole(wq_hbm, wqbuf, wqsem, 0)
    for u in range(AHEAD - 2):
        start_block(k_hbm, kbuf, ksem, u, rows=256)
        start_block(v_hbm, vbuf, vsem, u, rows=256)
    acc[...] = jnp.zeros(acc.shape, acc.dtype)

    for i in range(-2, 1):
        iteration(i)

    def body(i, carry):
        iteration(i)
        return carry
    lax.fori_loop(1, NU - AHEAD, body, 0)

    for i in range(NU - AHEAD, NU + 2):
        iteration(i)
    for b in range(B):
        o_copy(b).wait()


@jax.jit
def pallas_standalone__gqa_block_cached__near_ridge_kernel(
    x: jax.Array,
    k_cache: jax.Array,
    v_cache: jax.Array,
    wq: jax.Array,
    wo: jax.Array,
):
    assert x.shape == (B, SQ, D) and k_cache.shape == v_cache.shape == (B, HKV, SK, DH)
    assert wq.shape == (D, HQ * DH) and wo.shape == (HQ * DH, D)
    bf16, f32 = jnp.bfloat16, jnp.float32
    return pl.pallas_call(
        _kernel,
        in_specs=[pl.BlockSpec(memory_space=pltpu.HBM)] * 5,
        out_specs=pl.BlockSpec(memory_space=pltpu.HBM),
        out_shape=jax.ShapeDtypeStruct((B, SQ, D), bf16),
        scratch_shapes=[
            pltpu.VMEM((B, SQ, D), bf16),
            pltpu.VMEM((HKV, D, GW), bf16),
            pltpu.VMEM((HKV, D, GW), bf16),
            pltpu.VMEM((NS, SK, DH), bf16),
            pltpu.VMEM((NS, SK, DH), bf16),
            pltpu.VMEM((2, M, DH), bf16),
            pltpu.VMEM((2, M, SK), f32),
            pltpu.VMEM((2, M, 128), f32),
            pltpu.VMEM((2, SQ, GW), bf16),
            pltpu.VMEM((B, SQ, D), f32),
            pltpu.VMEM((B, SQ, D), bf16),
            pltpu.SemaphoreType.DMA((2,)),
            pltpu.SemaphoreType.DMA((HKV,)),
            pltpu.SemaphoreType.DMA((HKV,)),
            pltpu.SemaphoreType.DMA((NS,)),
            pltpu.SemaphoreType.DMA((NS,)),
            pltpu.SemaphoreType.DMA((B,)),
        ],
        compiler_params=pltpu.CompilerParams(vmem_limit_bytes=100 << 20,
                                             disable_bounds_checks=True),
    )(x, k_cache, v_cache, wq, wo.T)
```
